```python
import os as _os
_os.environ.setdefault('JAX_PLATFORMS', 'cpu')
import jax
import jax.numpy as jnp

def _softmax(x, axis=-1):
    return jax.nn.softmax(x, axis=axis)

def _gelu(x):
    return jax.nn.gelu(x, approximate=True)

def _silu(x):
    return jax.nn.silu(x)

def _sigmoid(x):
    return jax.nn.sigmoid(x)

def _layernorm(x, axis=-1, eps=1e-05):
    m = jnp.mean(x, axis=axis, keepdims=True)
    v = jnp.var(x, axis=axis, keepdims=True)
    return (x - m) / jnp.sqrt(v + eps)

def _scatter_add(tgt, idx, src, axis=0):
    return tgt.at[idx].add(src)

def _segment_sum(src, seg, n):
    return jax.ops.segment_sum(src, seg, n)

class _Rng:

    def __init__(self, key):
        self._k = key

    def _next(self):
        self._k, sub = jax.random.split(self._k)
        return sub

    def normal(self, shape):
        return jax.random.normal(self._next(), shape, dtype=jnp.bfloat16)

    def randint(self, lo, hi, shape):
        return jax.random.randint(self._next(), shape, lo, hi, dtype=jnp.int32)

    def uniform(self, shape, lo=0.0, hi=1.0):
        return jax.random.uniform(self._next(), shape, jnp.bfloat16, lo, hi)

    def permutation(self, n):
        return jax.random.permutation(self._next(), n)
kernel_name = 'adaLN_cond__softmax_full_mha__mixer_gmlp__prompt'

def setup_inputs():
    _rng = _Rng(jax.random.key(int.from_bytes(__import__("os").urandom(4), "little")))
    _w = lambda a: (lambda t: t.astype(jnp.bfloat16) if jnp.issubdtype(t.dtype, jnp.floating) else t)(jnp.asarray(a))

    def _A_setup():
        B, S, D = (1, 2048, 512)
        return {'x': _w((lambda *s: _rng.normal(s) * 0.05)(B, S, D)), 'wqkv': _w((lambda *s: _rng.normal(s) * 0.05)(D, 3 * D)), 'wo': _w((lambda *s: _rng.normal(s) * 0.05)(D, D))}
    _A_in = _A_setup()

    def _B_setup():
        B, S, D, F = (1, 2048, 512, 1792)
        Fh = F // 2
        return {'x': _w((lambda *s: _rng.normal(s) * 0.05)(B, S, D)), 'w_in': _w((lambda *s: _rng.normal(s) * 0.4)(D, 2 * Fh)), 'w_sp': _w(0.01 * (lambda *s: _rng.normal(s) * 0.4)(S, S)), 'b_sp': _w(1.0 + 0.01 * (lambda *s: _rng.normal(s) * 0.05)(S)), 'w_out': _w((lambda *s: _rng.normal(s) * 0.05)(Fh, D))}
    _B_in = _B_setup()
    return {'A_x': _A_in['x'], 'A_wqkv': _A_in['wqkv'], 'A_wo': _A_in['wo'], 'B_x': _B_in['x'], 'B_w_in': _B_in['w_in'], 'B_w_sp': _B_in['w_sp'], 'B_b_sp': _B_in['b_sp'], 'B_w_out': _B_in['w_out'], 'c': _w((lambda *s: _rng.normal(s) * 0.05)(1, 512) * 8.0), 'w_mod': _w((lambda *s: _rng.normal(s) * 0.05)(512, 6 * 512) * 512 ** (-0.5) * 8.0)}

def reference(A_x, A_wqkv, A_wo, B_x, B_w_in, B_w_sp, B_b_sp, B_w_out, c, w_mod):

    def _A_ref(x, wqkv, wo):
        B, S, D = x.shape
        H = 32
        Dh = D // H
        qkv = (lambda x, *d: x.transpose(*d))((x @ wqkv).reshape(B, S, 3, H, Dh), 2, 0, 3, 1, 4)
        q, k, v = (qkv[0], qkv[1], qkv[2])
        scale = Dh ** (-0.5)
        scores = jnp.einsum('bhqd,bhkd->bhqk', q, k) * scale
        p = _softmax(scores, axis=-1)
        o = jnp.einsum('bhqk,bhkd->bhqd', p, v)
        return (lambda x, *d: x.transpose(*d))(o, 0, 2, 1, 3).reshape(B, S, D) @ wo

    def _B_ref(x, w_in, w_sp, b_sp, w_out):
        B, S, D = x.shape
        F = w_in.shape[-1]
        Fh = F // 2
        z = _gelu(jnp.einsum('bsd,df->bsf', x, w_in))
        z1 = z[..., :Fh].copy()
        z2 = _layernorm(z[..., Fh:], axis=-1)
        g = jnp.einsum('ts,bsf->btf', w_sp, z2) + b_sp[None, :, None]
        return jnp.einsum('bsf,fd->bsd', z1 * g, w_out)
    x = A_x
    mod = (_silu(c) @ w_mod).reshape(c.shape[0], 6, 1, -1)
    sa, ca, ga, sb, cb, gb = (mod[:, 0].copy(), mod[:, 1].copy(), mod[:, 2].copy(), mod[:, 3].copy(), mod[:, 4].copy(), mod[:, 5].copy())
    h = _layernorm(x, axis=-1) * (1 + ca) + sa
    x = x + ga * _A_ref(h, A_wqkv, A_wo)
    h = _layernorm(x, axis=-1) * (1 + cb) + sb
    x = x + gb * _B_ref(h, B_w_in, B_w_sp, B_b_sp, B_w_out)
    return x
```

```python
import functools
import math

import jax
import jax.numpy as jnp
from jax import lax
import jax.experimental.pallas as pl
import jax.experimental.pallas.tpu as pltpu

S, D, H, DH = 2048, 512, 32, 16
F, FH = 1792, 896
EPS = 1e-5
F32, BF16 = jnp.float32, jnp.bfloat16
QSCALE = (DH ** -0.5) * math.log2(math.e)

T1 = 512
T3 = 512
T4 = 512
TQ = 512
CK = 128
NG = S // TQ
NC = S // CK
R8 = CK // 8


def _ln(x):
    m = jnp.mean(x, axis=-1, keepdims=True)
    xc = x - m
    v = jnp.mean(xc * xc, axis=-1, keepdims=True)
    return xc * lax.rsqrt(v + EPS)


def _gelu(z):
    c1 = math.sqrt(2.0 / math.pi)
    inner = z * (c1 + (c1 * 0.044715) * (z * z))
    hz = 0.5 * z
    return hz + hz * jnp.tanh(inner)


def _kernel(x_hbm, wqkv_hbm, wo_hbm, win_hbm, wsp_hbm, bsp_hbm, wout_hbm, c_hbm, wmod_hbm,
            out_hbm,
            x_v, wqkv_v, wo_v, win_v, wsp_v, bsp_v, wout_v, c_v, wmod_v,
            mod_v, wqvt_v, k_v, qt_v, vt_v, ot_v, s_a, s_b, m_a, m_b,
            x1_v, z1_v, z2_v, bcol_v, o_v, sems, xsems, osems):
    cp_c = pltpu.make_async_copy(c_hbm, c_v, sems.at[0])
    cp_m0 = pltpu.make_async_copy(wmod_hbm.at[:, pl.ds(0, 2 * D)], wmod_v.at[:, pl.ds(0, 2 * D)], sems.at[1])
    cp_qkv = pltpu.make_async_copy(wqkv_hbm, wqkv_v, sems.at[2])
    cp_x = [pltpu.make_async_copy(x_hbm.at[0, pl.ds(i * T1, T1), :], x_v.at[pl.ds(i * T1, T1), :], xsems.at[i])
            for i in range(S // T1)]
    cp_b = pltpu.make_async_copy(bsp_hbm, bsp_v, sems.at[3])
    cp_m1 = pltpu.make_async_copy(wmod_hbm.at[:, pl.ds(2 * D, 4 * D)], wmod_v.at[:, pl.ds(2 * D, 4 * D)], sems.at[4])
    cp_wo = pltpu.make_async_copy(wo_hbm, wo_v, sems.at[5])
    cp_win = pltpu.make_async_copy(win_hbm, win_v, sems.at[6])
    cp_wsp = pltpu.make_async_copy(wsp_hbm, wsp_v, sems.at[7])
    cp_wout = pltpu.make_async_copy(wout_hbm, wout_v, sems.at[8])
    for cp in [cp_c, cp_m0, cp_qkv] + cp_x + [cp_b, cp_m1, cp_wo, cp_win, cp_wsp, cp_wout]:
        cp.start()

    cp_c.wait()
    c = c_v[...].astype(F32)
    sc = jnp.broadcast_to(c * jax.nn.sigmoid(c), (16, D)).astype(BF16)
    cp_m0.wait()
    mod_v[:, pl.ds(0, 2 * D)] = jnp.dot(sc, wmod_v[:, pl.ds(0, 2 * D)], preferred_element_type=F32)[0:8]
    cp_qkv.wait()
    wqvt_v[pl.ds(0, D), :] = wqkv_v[:, pl.ds(0, D)].astype(F32).T.astype(BF16)
    wqvt_v[pl.ds(D, D), :] = wqkv_v[:, pl.ds(2 * D, D)].astype(F32).T.astype(BF16)

    for i in range(S // T1):
        cp_x[i].wait()

    def qkv_body(i, carry):
        rows = pl.ds(pl.multiple_of(i * T1, T1), T1)
        sa = mod_v[0:1, pl.ds(0, D)]
        ca = mod_v[0:1, pl.ds(D, D)]
        h = (_ln(x_v[rows, :].astype(F32)) * (1.0 + ca) + sa).astype(BF16)
        k_v[rows, :] = jnp.dot(h, wqkv_v[:, pl.ds(D, D)], preferred_element_type=F32).astype(BF16)
        qv = lax.dot_general(wqvt_v[...], h, (((1,), (1,)), ((), ())), preferred_element_type=F32)
        qt_v[:, rows] = (qv[0:D] * QSCALE).astype(BF16)
        vt_v[:, rows] = qv[D:2 * D].astype(BF16)
        return carry

    lax.fori_loop(0, S // T1, qkv_body, 0)

    cp_m1.wait()
    mod_v[:, pl.ds(2 * D, 4 * D)] = jnp.dot(sc, wmod_v[:, pl.ds(2 * D, 4 * D)], preferred_element_type=F32)[0:8]
    cp_b.wait()
    bsp = bsp_v[...].astype(F32)
    for i in range(S // 128):
        bcol_v[pl.ds(i * 128, 128), :] = jnp.broadcast_to(bsp[i:i + 1, :], (128, 128)).T

    def attn_step(h_qk, h_pv, s_w, m_w, s_r, m_r):
        if h_qk is not None:
            g = h_qk // 8
            j = h_qk % 8
            lanes = pl.ds(pl.multiple_of(g * 128, 128), 128)
        if h_pv is not None:
            hrows = pl.ds(pl.multiple_of(h_pv * DH, DH), DH)
        for cg in range(NG):
            cols = pl.ds(cg * TQ, TQ)
            if h_qk is not None:
                qg = qt_v[lanes, cols]
                rid = lax.broadcasted_iota(jnp.int32, (128, TQ), 0) // DH
                qm = jnp.where(rid == j, qg, jnp.zeros_like(qg))
                mx = None
            if h_pv is not None:
                m = m_r[:, cols]
                l = jnp.zeros((8, TQ), F32)
                acc = jnp.zeros((DH, TQ), F32)
            for c in range(NC):
                krows = pl.ds(c * CK, CK)
                if h_qk is not None:
                    s = jnp.dot(k_v[krows, lanes], qm, preferred_element_type=F32)
                    s_w[krows, cols] = s
                    for r in range(R8):
                        piece = s[r * 8:(r + 1) * 8]
                        mx = piece if mx is None else jnp.maximum(mx, piece)
                if h_pv is not None:
                    p = jnp.exp2(s_r[krows, cols].reshape(R8, 8, TQ) - m[None])
                    for r in reversed(range(R8)):
                        l = l + p[r]
                    pb = p.reshape(CK, TQ).astype(BF16)
                    acc = acc + jnp.dot(vt_v[hrows, krows], pb, preferred_element_type=F32)
            if h_qk is not None:
                m_w[:, cols] = jnp.broadcast_to(jnp.max(mx, axis=0, keepdims=True), (8, TQ))
            if h_pv is not None:
                lsum = jnp.sum(l, axis=0, keepdims=True)
                ot_v[hrows, cols] = acc * (1.0 / lsum)

    attn_step(0, None, s_a, m_a, None, None)

    def attn_body(i, carry):
        @pl.when(i % 2 == 0)
        def _():
            attn_step(i + 1, i, s_b, m_b, s_a, m_a)

        @pl.when(i % 2 == 1)
        def _():
            attn_step(i + 1, i, s_a, m_a, s_b, m_b)

        return carry

    lax.fori_loop(0, H - 1, attn_body, 0)
    attn_step(None, H - 1, None, None, s_b, m_b)

    cp_wo.wait()
    cp_win.wait()

    def mid_body(i, carry):
        rows = pl.ds(pl.multiple_of(i * T3, T3), T3)
        ga = mod_v[0:1, pl.ds(2 * D, D)]
        sb = mod_v[0:1, pl.ds(3 * D, D)]
        cb = mod_v[0:1, pl.ds(4 * D, D)]
        o = ot_v[:, rows].T.astype(BF16)
        y = jnp.dot(o, wo_v[...], preferred_element_type=F32)
        x1 = x_v[rows, :].astype(F32) + ga * y
        x1_v[rows, :] = x1
        h2 = (_ln(x1) * (1.0 + cb) + sb).astype(BF16)
        z = _gelu(jnp.dot(h2, win_v[...], preferred_element_type=F32))
        z1_v[rows, :] = z[:, 0:FH]
        z2_v[rows, :] = _ln(z[:, FH:F]).astype(BF16)
        return carry

    lax.fori_loop(0, S // T3, mid_body, 0)

    cp_wsp.wait()
    cp_wout.wait()

    def out_copy(i):
        rows = pl.ds(pl.multiple_of(i * T4, T4), T4)
        return pltpu.make_async_copy(o_v.at[rows, :], out_hbm.at[0, rows, :], osems.at[i])

    def out_body(i, carry):
        rows = pl.ds(pl.multiple_of(i * T4, T4), T4)
        gb = mod_v[0:1, pl.ds(5 * D, D)]
        g = jnp.dot(wsp_v[rows, :], z2_v[...], preferred_element_type=F32)
        bc = bcol_v[rows, :]
        g = g + jnp.concatenate([bc] * (FH // 128), axis=1)
        u = (z1_v[rows, :] * g).astype(BF16)
        y2 = jnp.dot(u, wout_v[...], preferred_element_type=F32)
        o_v[rows, :] = (x1_v[rows, :] + gb * y2).astype(BF16)
        out_copy(i).start()
        return carry

    lax.fori_loop(0, S // T4, out_body, 0)
    for i in range(S // T4):
        out_copy(i).wait()


@jax.jit
def pallas_adaLN_cond__softmax_full_mha__mixer_gmlp__prompt_kernel(
    A_x: jax.Array,
    A_wqkv: jax.Array,
    A_wo: jax.Array,
    B_x: jax.Array,
    B_w_in: jax.Array,
    B_w_sp: jax.Array,
    B_b_sp: jax.Array,
    B_w_out: jax.Array,
    c: jax.Array,
    w_mod: jax.Array,
):
    del B_x
    any_spec = pl.BlockSpec(memory_space=pl.ANY)
    scratch = [
        pltpu.VMEM((S, D), BF16),
        pltpu.VMEM((D, 3 * D), BF16),
        pltpu.VMEM((D, D), BF16),
        pltpu.VMEM((D, F), BF16),
        pltpu.VMEM((S, S), BF16),
        pltpu.VMEM((S // 128, 128), BF16),
        pltpu.VMEM((FH, D), BF16),
        pltpu.VMEM((1, D), BF16),
        pltpu.VMEM((D, 6 * D), BF16),
        pltpu.VMEM((8, 6 * D), F32),
        pltpu.VMEM((2 * D, D), BF16),
        pltpu.VMEM((S, D), BF16),
        pltpu.VMEM((D, S), BF16),
        pltpu.VMEM((D, S), BF16),
        pltpu.VMEM((D, S), F32),
        pltpu.VMEM((S, S), F32),
        pltpu.VMEM((S, S), F32),
        pltpu.VMEM((8, S), F32),
        pltpu.VMEM((8, S), F32),
        pltpu.VMEM((S, D), F32),
        pltpu.VMEM((S, FH), F32),
        pltpu.VMEM((S, FH), BF16),
        pltpu.VMEM((S, 128), F32),
        pltpu.VMEM((S, D), BF16),
        pltpu.SemaphoreType.DMA((9,)),
        pltpu.SemaphoreType.DMA((S // T1,)),
        pltpu.SemaphoreType.DMA((S // T4,)),
    ]
    return pl.pallas_call(
        _kernel,
        out_shape=jax.ShapeDtypeStruct((1, S, D), BF16),
        in_specs=[any_spec] * 9,
        out_specs=any_spec,
        scratch_shapes=scratch,
        compiler_params=pltpu.CompilerParams(vmem_limit_bytes=120 * 1024 * 1024),
        name="fused_block",
    )(A_x, A_wqkv, A_wo, B_w_in, B_w_sp, B_b_sp.reshape(S // 128, 128), B_w_out, c, w_mod)
```

```python
import contextlib
import functools
import math

import jax
import jax.numpy as jnp
from jax import lax
import jax.experimental.pallas as pl
import jax.experimental.pallas.tpu as pltpu

S, D, H, DH = 2048, 512, 32, 16
F, FH = 1792, 896
EPS = 1e-5
F32, BF16, U32 = jnp.float32, jnp.bfloat16, jnp.uint32
QSCALE = (DH ** -0.5) * math.log2(math.e)

T1 = 256
T3 = 256
T4 = 512
NSEM = 19
TQ = 512
CK = 128
NG = S // TQ
NC = S // CK
NCT = TQ // 128
N1, N3, N4 = S // T1, S // T3, S // T4
NI = NG * NC
NB = NC * 16 // 128
QR = 24
KT0 = (S // 128) * QR
TAIL = 3
RC = 16
QT_ROWS = 448
FS = 8
ZL = 2
L_MIN = 2.0 ** -70
L_MAX = 2.0 ** 20
PROFILE = False


def _scope(name):
    return jax.named_scope(name) if PROFILE else contextlib.nullcontext()


def _ln_parts(x):
    m = jnp.mean(x, axis=-1, keepdims=True)
    xc = x - m
    v = jnp.mean(xc * xc, axis=-1, keepdims=True)
    return xc, lax.rsqrt(v + EPS)


def _ln(x):
    xc, r = _ln_parts(x)
    return xc * r


def _gelu(z):
    c1 = math.sqrt(2.0 / math.pi)
    inner = z * (c1 + (c1 * 0.044715) * (z * z))
    hz = 0.5 * z
    return hz + hz * jnp.tanh(inner)


def _pack(x):
    return pltpu.bitcast(x.astype(BF16), U32)


def _unpack(x):
    return pltpu.bitcast(x, BF16)


def _rows(i, n):
    return pl.ds(i * n if isinstance(i, int) else pl.multiple_of(i * n, n), n)


def _kernel(x_hbm, wqkv_hbm, wo_hbm, win_hbm, wsp_hbm, bsp_hbm, wout_hbm, c_hbm, wmod_hbm,
            out_hbm,
            x_v, wqkv_v, wo_v, win_v, wsp_v, wout_v, wmod_v,
            mod_v, wqvt_v, h_v, k0_v, k_v, qt_v, vt_v, ot_v, p_a, p_b, l_a, l_b, lmin_v, lmax_v,
            ksel_v, qf_v, kb_a, kb_b,
            x1_v, z1_v, zr_v, z2_v, bcol_v, bsp_v, c_v, sems, osems):
    nsem = [0]

    def copies(src, dst, parts):
        out = []
        for idx in parts:
            out.append(pltpu.make_async_copy(src.at[idx], dst.at[idx], sems.at[nsem[0]]))
            nsem[0] += 1
        return out

    def rows_of(lo, hi, n):
        step = (hi - lo) // n
        return [(pl.ds(lo + i * step, step), slice(None)) for i in range(n)]

    full = [(slice(None), slice(None))]
    x2_hbm = x_hbm.at[0]
    cp_x = copies(x2_hbm, x_v, rows_of(0, S, N1))
    cp_c = copies(c_hbm, c_v, full)
    cp_m0 = copies(wmod_hbm, wmod_v, [(slice(None), pl.ds(0, 2 * D))])
    cp_wk = copies(wqkv_hbm, wqkv_v, [(slice(None), pl.ds(D, D))])
    cp_wqv = copies(wqkv_hbm, wqkv_v, [(slice(None), pl.ds(2 * D, D)), (slice(None), pl.ds(0, D))])
    cp_mid = ([pltpu.make_async_copy(bsp_hbm, bsp_v.at[pl.ds(0, S // 128), :], sems.at[NSEM - 1])]
              + copies(wmod_hbm, wmod_v, [(slice(None), pl.ds(2 * D, 4 * D))])
              + copies(wo_hbm, wo_v, full) + copies(win_hbm, win_v, full))
    cp_end = copies(wsp_hbm, wsp_v, full) + copies(wout_hbm, wout_v, full)
    assert nsem[0] == NSEM - 1

    def start(cps, priority=0):
        for cp in cps:
            cp.start(priority=priority)

    def wait(cps):
        for cp in cps:
            cp.wait()

    def kb_one(h, kb, x):
        b, d = x // DH, x % DH
        row = qf_v[h, pl.ds(KT0 + x, 8, stride=0), :]
        kb[d, pl.ds(b * 128, 128), :] = jnp.concatenate([row] * 16, axis=0).T

    with _scope('p1'):
        start(cp_x[:2] + cp_c + cp_m0 + cp_wk + cp_x[2:] + cp_wqv)
        start(cp_mid + cp_end, priority=1)
        wait(cp_x[:2])
        xn = [_ln(x_v[_rows(i, T1), :].astype(F32)) for i in range(2)]
        wait(cp_c + cp_m0)
        c = c_v[...].astype(F32)
        sc = jnp.broadcast_to(c * jax.nn.sigmoid(c), (16, D)).astype(BF16)
        mod0 = jnp.dot(sc, wmod_v[:, pl.ds(0, 2 * D)], preferred_element_type=F32)
        sa = mod0[0:1, 0:D]
        ca1 = 1.0 + mod0[0:1, D:2 * D]

        def hfun(i):
            xni = xn[i] if i < 2 else _ln(x_v[_rows(i, T1), :].astype(F32))
            return (xni * ca1 + sa).astype(BF16)

        kap = None
        hs = hfun(0)
        wait(cp_wk)
        for i in range(N1):
            if i == 1:
                wait(cp_x[2:4])
            if i == 3:
                wait(cp_x[4:])
            if i == N1 - 2:
                wait(cp_wqv)
                wqvt_v[pl.ds(0, D // 2), :] = pltpu.bitcast(wqkv_v[:, pl.ds(2 * D, D)].T, U32)
                wqvt_v[pl.ds(D // 2, D // 2), :] = pltpu.bitcast(wqkv_v[:, pl.ds(0, D)].T, U32)
            hn = hfun(i + 1) if i + 1 < N1 else None
            half = _rows(i, T1 // 2)
            h_v[half, :] = pltpu.bitcast(hs, U32)
            kf = jnp.dot(hs, wqkv_v[:, pl.ds(D, D)], preferred_element_type=F32)
            ka = jnp.max(jnp.abs(kf).reshape(T1 // 8, 8, D), axis=0)
            kap = ka if kap is None else jnp.maximum(kap, ka)
            for cc in range(T1 // CK):
                ksel_v[pl.ds((i * (T1 // CK) + cc) * 16, 16), :] = kf[cc * CK:cc * CK + 16]
            k0_v[half, :] = _pack(kf)
            hs = hn
        kcol = jnp.broadcast_to(jnp.max(kap, axis=0, keepdims=True), (128, D)).T
        for b in range(NB):
            qf_v[0:H, pl.ds(KT0 + b * DH, DH), :] = ksel_v[pl.ds(b * 128, 128), :].T.reshape(H, DH, 128)
        qf_v[0:H, pl.ds(KT0 + NB * DH, 8), :] = jnp.zeros((H, 8, 128), F32)
        for x in range(NB * DH):
            kb_one(0, kb_a, x)
        lane = lax.broadcasted_iota(jnp.int32, (S // 2, 128), 1)
        for g in range(D // 128):
            kg = k0_v[:, pl.ds(g * 128, 128)]
            for j in range(8):
                kr = kg if j == 0 else pltpu.roll(kg, 128 - DH * j, 1)
                k_v[g * 8 + j] = jnp.where(lane == DH, jnp.uint32(0x3F803F80), kr)

        def proj_t(part, i):
            return lax.dot_general(_unpack(wqvt_v[pl.ds(part * D // 2, D // 2), :]),
                                   _unpack(h_v[_rows(i, T1 // 2), :]),
                                   (((1,), (1,)), ((), ())), preferred_element_type=F32)

        for i in range(N1):
            vt_v[:, _rows(i, T1)] = _pack(proj_t(0, i))
        rid = lax.broadcasted_iota(jnp.int32, (H, DH, 128), 1)
        for i in range(N1):
            qt = proj_t(1, i)
            for ct in range(T1 // 128):
                q = qt[:, ct * 128:(ct + 1) * 128] * QSCALE
                bound = jnp.sum((jnp.abs(q) * kcol).reshape(H, DH, 128), axis=1, keepdims=True)
                shift = (bound * -1.02).astype(BF16).astype(F32)
                aug = jnp.where(rid == 0, jnp.broadcast_to(shift, (H, DH, 128)), 0.0)
                full_q = jnp.concatenate([q.reshape(H, DH, 128), aug], axis=1)
                gct = i * (T1 // 128) + ct
                qf_v[0:H, pl.ds(gct * QR, QR), :] = full_q[:, 0:QR]
                qt_v[:, :, pl.ds(gct * 128, 128)] = _pack(full_q.reshape(H * 2 * DH, 128)).reshape(H, DH, 128)
        lmin_v[...] = jnp.full((8, S), 1.0, F32)
        lmax_v[...] = jnp.full((8, S), 1.0, F32)

    gaps = [(it, g) for it in range(NI - TAIL) for g in range(7)]
    steps = [(cg, c, d) for cg in range(NG) for c in range(NC) for d in range(DH)]
    plan = {}
    for i, sp in enumerate(steps):
        plan.setdefault(gaps[i * len(gaps) // len(steps)], []).append(sp)

    def qk_items(h, hd, kb, p_w, l_w, h3, kb3):
        st = {}

        def vstep(cg, c, d):
            def qrow(r):
                return jnp.concatenate(
                    [qf_v[hd, pl.ds((cg * NCT + ct) * QR + r, 8, stride=0), :] for ct in range(NCT)], axis=1)

            qr = qrow(d)
            prev = [qrow(DH)] * 2 if d == 0 else st['ac']
            st['ac'] = [prev[u] + jnp.concatenate([kb[d, pl.ds(c * 16 + u * 8, 8), :]] * NCT, axis=1) * qr
                        for u in range(2)]
            if d == DH - 1:
                pp = [jnp.exp2(a) for a in st['ac']]
                pcols = pl.ds(cg * TQ, TQ)
                p_w[pl.ds(c * CK // 2, 8), pcols] = _pack(jnp.concatenate(pp, axis=0))
                x = pp[0] + pp[1]
                st['l2'] = x if c == 0 else st['l2'] + x
                if c == NC - 1:
                    l_w[pl.ds(8, 8), pcols] = st['l2']

        def item(cg, c):
            cols = pl.ds(cg * TQ, TQ)
            if c == 0:
                st['q'] = qt_v[h, :, cols]
                st['l'] = None
            kc = _unpack(k_v[h, pl.ds(c * CK // 2 + 8, 56), :])
            s = jnp.dot(kc[:, 0:2 * DH], _unpack(st['q']), preferred_element_type=F32)
            it = cg * NC + c
            for g in range(7):
                sg = s[g * 16:(g + 1) * 16]
                p = jnp.exp2(sg)
                p_w[pl.ds(c * CK // 2 + (g + 1) * 8, 8), cols] = _pack(p)
                l = p[0:8] if st['l'] is None else st['l'] + p[0:8]
                st['l'] = l + p[8:16]
                todo = plan.get((it, g), [])
                if todo:
                    qf_v[H, 0:8, :] = sg[0:8, 0:128]
                for sp in todo:
                    vstep(*sp)
                if g == 3 and it < NI - TAIL:
                    nx = NB * DH
                    for x in range(it * nx // (NI - TAIL), (it + 1) * nx // (NI - TAIL)):
                        kb_one(h3, kb3, x)
            if c == NC - 1:
                l_w[pl.ds(0, 8), cols] = st['l']

        return [functools.partial(item, cg, c) for cg in range(NG) for c in range(NC)]

    def pv_items(h, p_r, l_r, track=True):
        st = {}

        def item(cg, c):
            cols = pl.ds(cg * TQ, TQ)
            pb = _unpack(p_r[pl.ds(c * CK // 2, CK // 2), cols])
            o = jnp.dot(_unpack(vt_v[_rows(h, 8), pl.ds(c * CK, CK)]), pb, preferred_element_type=F32)
            st['acc'] = o if c == 0 else o + st['acc']
            if c == NC - 1:
                lsum = jnp.sum(l_r[0:8, cols] + l_r[8:16, cols], axis=0, keepdims=True)
                ot_v[_rows(h, DH), cols] = st['acc'] * (1.0 / lsum)
                if track:
                    lmin_v[0:1, cols] = jnp.minimum(lmin_v[0:1, cols], lsum)
                    lmax_v[0:1, cols] = jnp.maximum(lmax_v[0:1, cols], lsum)

        return [functools.partial(item, cg, c) for cg in range(NG) for c in range(NC)]

    def attn_step(h, w, r, kb_next):
        qk = qk_items(h + 1, h + 1, *w, jnp.minimum(h + 2, H - 1), kb_next)
        for a, b in zip(qk, pv_items(h, *r)):
            a()
            b()

    with _scope('p2_first'):
        zero = jnp.minimum(jnp.min(kap), 0.0).astype(jnp.int32)
        for it in qk_items(0, jnp.clip(zero, 0, H), kb_a, p_a, l_a, jnp.clip(zero + 1, 0, H), kb_b):
            it()

    def attn_body(i, carry):
        @pl.when(i % 2 == 0)
        def _():
            attn_step(i, (kb_b, p_b, l_b), (p_a, l_a), kb_a)

        @pl.when(i % 2 == 1)
        def _():
            attn_step(i, (kb_a, p_a, l_a), (p_b, l_b), kb_b)

        return carry

    with _scope('p2_loop'):
        lax.fori_loop(0, H - 1, attn_body, 0)

    l_last = jnp.sum(l_b[0:8, :] + l_b[8:16, :], axis=0, keepdims=True)
    lo = jnp.min(jnp.minimum(lmin_v[0:1, :], l_last))
    hi = jnp.max(jnp.maximum(lmax_v[0:1, :], l_last))
    safe = jnp.logical_and(lo >= L_MIN, hi <= L_MAX)

    @pl.when(jnp.logical_not(safe))
    def _():
        def exact(t, carry):
            h = t // NG
            cols = _rows(t % NG, TQ)
            q = _unpack(qt_v[h, 0:8, cols])
            s = jnp.dot(_unpack(k_v[h])[:, 0:DH], q, preferred_element_type=F32)
            p = jnp.exp2(s - jnp.max(s, axis=0, keepdims=True))
            p_b[:, cols] = _pack(p)
            l = jnp.sum(p.reshape(S // 8, 8, TQ), axis=0)
            l_b[0:8, cols] = l
            l_b[8:16, cols] = jnp.zeros((8, TQ), F32)
            o = jnp.dot(_unpack(vt_v[_rows(h, 8), :]), p.astype(BF16), preferred_element_type=F32)
            ot_v[_rows(h, DH), cols] = o * (1.0 / jnp.sum(l, axis=0, keepdims=True))
            return carry

        lax.fori_loop(0, H * NG, exact, 0)

    KA = D - 128
    zoff = jnp.minimum(lo, 0.0).astype(jnp.int32) * 16

    def paced(r0):
        return pl.ds(pl.multiple_of(jnp.clip(zoff + r0, 0, S), 16), RC)

    NZ = FH // 128
    nch = T3 // RC
    md = {}

    def modrow(k):
        return jnp.concatenate([md[k * 4 + t] for t in range(4)], axis=1)

    def wo_rest(i):
        rows = pl.ds(i * T3, T3)
        ob = ot_v[pl.ds(KA, D - KA), rows].T.astype(BF16)
        return jnp.dot(ob, wo_v[pl.ds(KA, D - KA), :], preferred_element_type=F32)

    def front_chunk(i, yb, j):
        r0 = i * T3 + j * RC
        x1 = x1_v[paced(r0) if i > 0 else pl.ds(r0, RC), :] + modrow(0) * yb[j * RC:(j + 1) * RC]
        x1_v[pl.ds(r0, RC), :] = x1
        return (_ln(x1) * (1.0 + modrow(2)) + modrow(1)).astype(BF16)

    with _scope('p2_last'):
        wait(cp_mid)
        c = c_v[...].astype(F32)
        sc = jnp.broadcast_to(c * jax.nn.sigmoid(c), (16, D)).astype(BF16)
        bsp = bsp_v[0:S // 128, :].astype(F32)
        for i in range(S // 128):
            bcol_v[pl.ds(i * 128, 128), :] = jnp.broadcast_to(bsp[i:i + 1, :], (128, 128)).T
        last = pv_items(H - 1, p_b, l_b, track=False)
        ys = {}

        def mod_piece(t):
            mt = jnp.dot(sc, wmod_v[:, pl.ds(2 * D + t * 128, 128)], preferred_element_type=F32)
            md[t] = mt[0:1]
            if t >= 12:
                mod_v[0:8, pl.ds((t - 12) * 128, 128)] = mt[0:8]

        def wo_piece(i, kt):
            rows = pl.ds(i * 128, 128)
            oa = ot_v[pl.ds(kt * 128, 128), rows].T.astype(BF16)
            ya = jnp.dot(oa, wo_v[pl.ds(kt * 128, 128), :], preferred_element_type=F32)
            ys[i] = ya if kt == 0 else ya + ys[i]

        def x1_part(i):
            rows = pl.ds(i * 128, 128)
            x1_v[rows, :] = x_v[rows, :].astype(F32) + modrow(0) * ys.pop(i)

        for n, it in enumerate(last):
            it()
            if n % 4 == 0:
                mod_piece(n // 4)
            else:
                wo_piece(n // 4, n % 4 - 1)
            if n % 4 == 3 and n // 4 >= 3:
                for i in (range(4) if n // 4 == 3 else [n // 4]):
                    x1_part(i)
            if n == 47:
                yb = wo_rest(0)
                h2 = jnp.concatenate([front_chunk(0, yb, j) for j in range(nch)], axis=0)

    with _scope('p3'):
        for i in range(N3):
            rows = pl.ds(i * T3, T3)
            yb = wo_rest(i + 1) if i + 1 < N3 else None
            hparts = []
            for sl in range(2 * NZ):
                lhs = h2
                if sl == NZ + ZL:
                    tok = pltpu.bitcast(jnp.broadcast_to(jnp.max(rstd, axis=0, keepdims=True) * 0.0, (8, 128)), U32)
                    h32 = pltpu.bitcast(h2, U32)
                    lhs = _unpack(jnp.concatenate(
                        [jnp.concatenate([h32[0:8, 0:128] + tok, h32[0:8, 128:]], axis=1), h32[8:]], axis=0))
                zraw = jnp.dot(lhs, win_v[:, pl.ds(((sl + NZ) % (2 * NZ)) * 128, 128)], preferred_element_type=F32)
                zt = _gelu(zraw)
                if sl < NZ:
                    zr_v[rows, pl.ds(sl * 128, 128)] = zt
                    s1 = zt if sl == 0 else s1 + zt
                    s2 = zt * zt if sl == 0 else s2 + zt * zt
                    if sl == NZ - 1:
                        mean = jnp.sum(s1, axis=-1, keepdims=True) * (1.0 / FH)
                        var = jnp.sum(s2, axis=-1, keepdims=True) * (1.0 / FH) - mean * mean
                        rstd = lax.rsqrt(jnp.maximum(var, 0.0) + EPS)
                else:
                    z1_v[rows, pl.ds((sl - NZ) * 128, 128)] = zt
                    lo_s = NZ + ZL
                    if sl >= lo_s:
                        zr_v[pl.ds(S, 8), pl.ds(0, 128)] = zraw[0:8]
                        ns = 2 * NZ - lo_s
                        for j in range((sl - lo_s) * nch // ns, (sl - lo_s + 1) * nch // ns):
                            r0 = i * T3 + j * RC
                            g2 = zr_v[paced(r0), :]
                            z2_v[pl.ds(r0 // 2, RC // 2), :] = _pack(
                                (g2 - mean[j * RC:(j + 1) * RC]) * rstd[j * RC:(j + 1) * RC])
                if yb is not None and sl < FS:
                    x1_v[pl.ds(S, 8), pl.ds(0, 128)] = zraw[0:8]
                    for j in range(sl * nch // FS, (sl + 1) * nch // FS):
                        hparts.append(front_chunk(i + 1, yb, j))
            if yb is not None:
                h2 = jnp.concatenate(hparts, axis=0)

    TO = T4 // 2

    def out_copy(i):
        rows = _rows(i, TO)
        return pltpu.make_async_copy(x_v.at[rows, :], out_hbm.at[0, rows, :], osems.at[i])

    def out_body(i, carry):
        rows = _rows(i, T4)
        g = jnp.dot(wsp_v[rows, :], _unpack(z2_v[...]), preferred_element_type=F32)
        bc = bcol_v[rows, :]
        g = g + jnp.concatenate([bc] * (FH // 128), axis=1)
        u = (z1_v[rows, :] * g).astype(BF16)
        for t in range(2):
            hrows = _rows(2 * i + t, TO)
            y2 = jnp.dot(u[t * TO:(t + 1) * TO], wout_v[...], preferred_element_type=F32)
            x_v[hrows, :] = (x1_v[hrows, :] + mod_v[0:1, :] * y2).astype(BF16)
            out_copy(2 * i + t).start()
        return carry

    with _scope('p4'):
        wait(cp_end)
        lax.fori_loop(0, N4, out_body, 0)
        for i in range(2 * N4):
            out_copy(i).wait()


@jax.jit
def pallas_adaLN_cond__softmax_full_mha__mixer_gmlp__prompt_kernel(
    A_x: jax.Array,
    A_wqkv: jax.Array,
    A_wo: jax.Array,
    B_x: jax.Array,
    B_w_in: jax.Array,
    B_w_sp: jax.Array,
    B_b_sp: jax.Array,
    B_w_out: jax.Array,
    c: jax.Array,
    w_mod: jax.Array,
):
    del B_x
    any_spec = pl.BlockSpec(memory_space=pl.ANY)
    scratch = [
        pltpu.VMEM((S, D), BF16),
        pltpu.VMEM((D, 3 * D), BF16),
        pltpu.VMEM((D, D), BF16),
        pltpu.VMEM((D, F), BF16),
        pltpu.VMEM((S, S), BF16),
        pltpu.VMEM((FH, D), BF16),
        pltpu.VMEM((D, 6 * D), BF16),
        pltpu.VMEM((32, D), F32),
        pltpu.VMEM((D, D), U32),
        pltpu.VMEM((S // 2, D), U32),
        pltpu.VMEM((S // 2, D), U32),
        pltpu.VMEM((H, S // 2, 128), U32),
        pltpu.VMEM((H, DH, S), U32),
        pltpu.VMEM((D // 2, S), U32),
        pltpu.VMEM((D, S), F32),
        pltpu.VMEM((S // 2, S), U32),
        pltpu.VMEM((S // 2, S), U32),
        pltpu.VMEM((16, S), F32),
        pltpu.VMEM((16, S), F32),
        pltpu.VMEM((8, S), F32),
        pltpu.VMEM((8, S), F32),
        pltpu.VMEM((NB * 128, D), F32),
        pltpu.VMEM((H + 2, QT_ROWS, 128), F32),
        pltpu.VMEM((DH, NB * 128, 128), F32),
        pltpu.VMEM((DH, NB * 128, 128), F32),
        pltpu.VMEM((S + 32, D), F32),
        pltpu.VMEM((S, FH), F32),
        pltpu.VMEM((S + 128, FH), F32),
        pltpu.VMEM((S // 2, FH), U32),
        pltpu.VMEM((S, 128), F32),
        pltpu.VMEM((248, 128), BF16),
        pltpu.VMEM((1, D), BF16),
        pltpu.SemaphoreType.DMA((NSEM,)),
        pltpu.SemaphoreType.DMA((2 * N4,)),
    ]
    return pl.pallas_call(
        _kernel,
        out_shape=jax.ShapeDtypeStruct((1, S, D), BF16),
        in_specs=[any_spec] * 9,
        out_specs=any_spec,
        scratch_shapes=scratch,
        compiler_params=pltpu.CompilerParams(vmem_limit_bytes=124 * 1024 * 1024),
        name="fused_block",
    )(A_x, A_wqkv, A_wo, B_w_in, B_w_sp, B_b_sp.reshape(S // 128, 128), B_w_out, c, w_mod)
```

```python
import contextlib
import functools
import math

import jax
import jax.numpy as jnp
from jax import lax
import jax.experimental.pallas as pl
import jax.experimental.pallas.tpu as pltpu

S, D, H, DH = 2048, 512, 32, 16
F, FH = 1792, 896
EPS = 1e-5
F32, BF16, U32 = jnp.float32, jnp.bfloat16, jnp.uint32
QSCALE = (DH ** -0.5) * math.log2(math.e)

T1 = 256
T3 = 256
T4 = 512
TQ = 512
CK = 128
NG = S // TQ
NC = S // CK
NCT = TQ // 128
N1, N3, N4 = S // T1, S // T3, S // T4
NI = NG * NC
NB = NC * 16 // 128
QR = 24
KT0 = (S // 128) * QR
TAIL = 2
KBG = 6
HS = 9
PAT = 3222322
PAT2 = 3232322
PER = 3
TO = 128
RC = 16
QT_ROWS = 448
NQB = 3 * (S // 128)
QB_ROWS = 576
FS = 8
ZL = 2
L_MIN = 2.0 ** -70
L_MAX = 2.0 ** 20
PROFILE = False


def _scope(name):
    return jax.named_scope(name) if PROFILE else contextlib.nullcontext()


def _ln(x):
    m = jnp.mean(x, axis=-1, keepdims=True)
    xc = x - m
    v = jnp.mean(xc * xc, axis=-1, keepdims=True)
    return xc * lax.rsqrt(v + EPS)


def _gelu(z):
    c1 = math.sqrt(2.0 / math.pi)
    inner = z * (c1 + (c1 * 0.044715) * (z * z))
    hz = 0.5 * z
    return hz + hz * jnp.tanh(inner)


def _pack(x):
    return pltpu.bitcast(x.astype(BF16), U32)


def _unpack(x):
    return pltpu.bitcast(x, BF16)


def _rows(i, n):
    return pl.ds(i * n if isinstance(i, int) else pl.multiple_of(i * n, n), n)


def _kernel(x_hbm, wqkv_hbm, wo_hbm, win_hbm, wsp_hbm, bsp_hbm, wout_hbm, c_hbm, wmod_hbm,
            out_hbm,
            x_v, wqkv_v, wo_v, win_v, wsp_v, wout_v, wmod_v,
            mod_v, wqvt_v, h_v, k0_v, k_v, qt_v, vt_v, ot_v, p_a, p_b, l_a, l_b, lmin_v, lmax_v,
            ksel_v, qf_v, kb_a, kb_b, qb_a, qb_b,
            x1_v, z1_v, zr_v, z2_v, bcol_v, bsp_v, c_v, sems):
    def copies(sem, src, dst, parts):
        return [pltpu.make_async_copy(src.at[idx], dst.at[idx], sems.at[sem]) for idx in parts]

    def cols_of(lo, n):
        return [(slice(None), pl.ds(lo, n))]

    full = [(slice(None), slice(None))]
    xsem = [0, 1, 1, 9, 2, 2, 10, 10]
    cp_x = [copies(xsem[i], x_hbm.at[0], x_v, [(pl.ds(i * T1, T1), slice(None))])[0] for i in range(N1)]
    cp_ca = copies(3, c_hbm, c_v, full) + copies(3, wmod_hbm, wmod_v, cols_of(D, D))
    cp_sa = copies(9, wmod_hbm, wmod_v, cols_of(0, D))
    cp_wk = copies(4, wqkv_hbm, wqkv_v, cols_of(D, D))
    cp_wqv = copies(5, wqkv_hbm, wqkv_v, cols_of(2 * D, D) + cols_of(0, D))
    cp_mid = ([pltpu.make_async_copy(bsp_hbm, bsp_v.at[pl.ds(0, S // 128), :], sems.at[6])]
              + copies(6, wmod_hbm, wmod_v, cols_of(2 * D, 4 * D))
              + copies(6, wo_hbm, wo_v, full) + copies(6, win_hbm, win_v, full))
    cp_end = copies(7, wsp_hbm, wsp_v, full) + copies(7, wout_hbm, wout_v, full)

    def start(cps, priority=0):
        for cp in cps:
            cp.start(priority=priority)

    def wait(cps):
        for cp in cps:
            cp.wait()

    def kb_one(h, kb, x):
        b, d = x // DH, x % DH
        row = jnp.broadcast_to(qf_v[h, pl.ds(KT0 + x, 1), :], (8, 128))
        kb[d, pl.ds(b * 128, 128), :] = jnp.concatenate([row] * 16, axis=0).T

    def qb_one(h, qb, x):
        ct, part = x // 3, x % 3
        blk = qf_v[h, pl.ds(ct * QR + part * 8, 8), :]
        for r in range(part * 8, min(part * 8 + 8, DH + 1)):
            qb[pl.ds(((ct // NCT) * (DH + 1) + r) * 8, 8), pl.ds((ct % NCT) * 128, 128)] = (
                jnp.broadcast_to(blk[r % 8:r % 8 + 1], (8, 128)))

    with _scope('p1'):
        start(cp_x[:1] + cp_ca + cp_wk + cp_x[1:3] + cp_sa + cp_x[3:] + cp_wqv)
        start(cp_mid + cp_end, priority=1)
        zero = lax.fori_loop(0, 4, lambda i, z: jnp.minimum(z, i), jnp.int32(0))
        wk = lambda: wqkv_v[:, pl.ds(D, D)]
        xnorm = lambda i: _ln(x_v[_rows(i, T1), :].astype(F32))
        kst = {'kap': None}

        def k_done(i, hs, kf):
            half = _rows(i, T1 // 2)
            h_v[half, :] = pltpu.bitcast(hs, U32)
            ka = jnp.max(jnp.abs(kf).reshape(T1 // 8, 8, D), axis=0)
            kst['kap'] = ka if kst['kap'] is None else jnp.maximum(kst['kap'], ka)
            for cc in range(T1 // CK):
                ksel_v[pl.ds((i * (T1 // CK) + cc) * 16, 16), :] = kf[cc * CK:cc * CK + 16]
            k0_v[half, :] = _pack(kf)

        wait(cp_x[:1])
        xn0 = xnorm(0)
        wait(cp_ca)
        c = c_v[...].astype(F32)
        sc = jnp.broadcast_to(c * jax.nn.sigmoid(c), (16, D)).astype(BF16)
        ca1 = 1.0 + jnp.dot(sc, wmod_v[:, pl.ds(D, D)], preferred_element_type=F32)[0:1]
        early = [xn0 * ca1]
        lhs0 = early[0].astype(BF16)
        wait(cp_wk)
        x1_v[_rows(0, T1), :] = jnp.dot(lhs0, wk(), preferred_element_type=F32)
        wait(cp_x[1:3])
        early.append(xnorm(1) * ca1)
        x1_v[_rows(1, T1), :] = jnp.dot(early[1].astype(BF16), wk(), preferred_element_type=F32)
        xs = xnorm(2) * ca1
        wait(cp_sa + cp_x[3:4])
        sa16 = jnp.dot(sc, wmod_v[:, pl.ds(0, D)], preferred_element_type=F32)
        sa = sa16[0:1]
        hs = (xs + sa).astype(BF16)
        for i in range(2, N1):
            if i == 3:
                wait(cp_x[4:6])
            if i == 5:
                wait(cp_x[6:])
            if i == N1 - 1:
                wait(cp_wqv)
                wqvt_v[pl.ds(0, D // 2), :] = pltpu.bitcast(wqkv_v[:, pl.ds(2 * D, D)].T, U32)
                wqvt_v[pl.ds(D // 2, D // 2), :] = pltpu.bitcast(wqkv_v[:, pl.ds(0, D)].T, U32)
            hn = (xnorm(i + 1) * ca1 + sa).astype(BF16) if i + 1 < N1 else None
            k_done(i, hs, jnp.dot(hs, wk(), preferred_element_type=F32))
            if i == 3:
                kbias = jnp.dot(sa16.astype(BF16), wk(), preferred_element_type=F32)[0:1]
                for e in range(2):
                    k_done(e, (early[e] + sa).astype(BF16), x1_v[_rows(e, T1), :] + kbias)
            hs = hn
        kap = kst['kap']
        kcol = jnp.broadcast_to(jnp.max(kap, axis=0, keepdims=True), (128, D)).T
        for b in range(NB):
            qf_v[0:H, pl.ds(KT0 + b * DH, DH), :] = ksel_v[pl.ds(b * 128, 128), :].T.reshape(H, DH, 128)
        for x in range(NB * DH):
            kb_one(0, kb_a, x)
        lane = lax.broadcasted_iota(jnp.int32, (S // 2, 128), 1)
        for g in range(D // 128):
            kg = k0_v[:, pl.ds(g * 128, 128)]
            for j in range(8):
                kr = kg if j == 0 else pltpu.roll(kg, 128 - DH * j, 1)
                k_v[g * 8 + j] = jnp.where(lane == DH, jnp.uint32(0x3F803F80), kr)

        def proj_t(part, i):
            return lax.dot_general(_unpack(wqvt_v[pl.ds(part * D // 2, D // 2), :]),
                                   _unpack(h_v[_rows(i, T1 // 2), :]),
                                   (((1,), (1,)), ((), ())), preferred_element_type=F32)

        for i in range(N1):
            vt_v[:, _rows(i, T1)] = _pack(proj_t(0, i))
        rid = lax.broadcasted_iota(jnp.int32, (H, DH, 128), 1)
        for i in range(N1):
            qt = proj_t(1, i)
            for ct in range(T1 // 128):
                q = qt[:, ct * 128:(ct + 1) * 128] * QSCALE
                bound = jnp.sum((jnp.abs(q) * kcol).reshape(H, DH, 128), axis=1, keepdims=True)
                shift = (bound * -1.02).astype(BF16).astype(F32)
                aug = jnp.where(rid == 0, jnp.broadcast_to(shift, (H, DH, 128)), 0.0)
                full_q = jnp.concatenate([q.reshape(H, DH, 128), aug], axis=1)
                gct = i * (T1 // 128) + ct
                qf_v[0:H, pl.ds(gct * QR, QR), :] = full_q[:, 0:QR]
                qt_v[:, :, pl.ds(gct * 128, 128)] = _pack(full_q.reshape(H * 2 * DH, 128)).reshape(H, DH, 128)
        for x in range(NQB):
            qb_one(0, qb_a, x)
        lmin_v[...] = jnp.full((8, S), 1.0, F32)
        lmax_v[...] = jnp.full((8, S), 1.0, F32)

    z8 = pl.multiple_of(zero * 8, 8)
    steps = [(cg, c, d) for cg in range(NG) for c in range(NC) for d in range(DH)]
    slots = [(0, -1)] * HS
    for it in range(NI):
        pat = str(PAT2 if it % PER == 0 else PAT)
        slots += [(it, g) for g in range(7) for _ in range(int(pat[g]))]
    assert len(slots) >= len(steps)
    plan = {}
    for sl, sp in zip(slots, steps):
        plan.setdefault(sl, []).append(sp)

    def qk_items(h, kb, qb, p_w, l_w, h3, kb3, qb3):
        st = {}

        def vstep(cg, c, d):
            def qrow(r):
                return qb[pl.ds(z8 + (cg * (DH + 1) + r) * 8, 8), :]

            qr = qrow(d)
            prev = [qrow(DH)] * 2 if d == 0 else st['ac']
            st['ac'] = [prev[u] + jnp.concatenate([kb[d, pl.ds(c * 16 + u * 8, 8), :]] * NCT, axis=1) * qr
                        for u in range(2)]
            if d == DH - 1:
                pp = [jnp.exp2(a) for a in st['ac']]
                pcols = pl.ds(cg * TQ, TQ)
                p_w[pl.ds(c * CK // 2, 8), pcols] = _pack(jnp.concatenate(pp, axis=0))
                x = pp[0] + pp[1]
                st['l2'] = x if c == 0 else st['l2'] + x
                if c == NC - 1:
                    l_w[pl.ds(8, 8), pcols] = st['l2']

        def item(cg, c):
            cols = pl.ds(cg * TQ, TQ)
            if c == 0:
                st['q'] = qt_v[h, :, cols]
                st['l'] = None
            kc = _unpack(k_v[h, pl.ds(c * CK // 2 + 8, 56), :])
            s = jnp.dot(kc[:, 0:2 * DH], _unpack(st['q']), preferred_element_type=F32)
            it = cg * NC + c
            for sp in plan.get((it, -1), []):
                vstep(*sp)
            for g in range(7):
                sg = s[g * 16:(g + 1) * 16]
                p = jnp.exp2(sg)
                p_w[pl.ds(c * CK // 2 + (g + 1) * 8, 8), cols] = _pack(p)
                l = p[0:8] if st['l'] is None else st['l'] + p[0:8]
                st['l'] = l + p[8:16]
                todo = plan.get((it, g), [])
                if todo:
                    qb[pl.ds(QB_ROWS - 8, 8), pl.ds(0, 128)] = sg[0:8, 0:128]
                for sp in todo:
                    vstep(*sp)
                if g == KBG and it < NI - TAIL:
                    qf_v[H, 0:8, :] = sg[0:8, 0:128]
                    for nx, build, dst in ((NB * DH, kb_one, kb3), (NQB, qb_one, qb3)):
                        for x in range(it * nx // (NI - TAIL), (it + 1) * nx // (NI - TAIL)):
                            build(h3, dst, x)
            if c == NC - 1:
                l_w[pl.ds(0, 8), cols] = st['l']

        return [functools.partial(item, cg, c) for cg in range(NG) for c in range(NC)]

    def pv_items(h, p_r, l_r, track=True):
        st = {}

        def item(cg, c):
            cols = pl.ds(cg * TQ, TQ)
            pb = _unpack(p_r[pl.ds(c * CK // 2, CK // 2), cols])
            o = jnp.dot(_unpack(vt_v[_rows(h, 8), pl.ds(c * CK, CK)]), pb, preferred_element_type=F32)
            st['acc'] = o if c == 0 else o + st['acc']
            if c == NC - 1:
                lsum = jnp.sum(l_r[0:8, cols] + l_r[8:16, cols], axis=0, keepdims=True)
                ot_v[_rows(h, DH), cols] = st['acc'] * (1.0 / lsum)
                if track:
                    lmin_v[0:1, cols] = jnp.minimum(lmin_v[0:1, cols], lsum)
                    lmax_v[0:1, cols] = jnp.maximum(lmax_v[0:1, cols], lsum)

        return [functools.partial(item, cg, c) for cg in range(NG) for c in range(NC)]

    def attn_step(h, w, r, nxt):
        qk = qk_items(h + 1, *w, jnp.minimum(h + 2, H - 1), *nxt)
        for a, b in zip(qk, pv_items(h, *r)):
            a()
            b()

    with _scope('p2_first'):
        for it in qk_items(0, kb_a, qb_a, p_a, l_a, zero + 1, kb_b, qb_b):
            it()

    def attn_body(i, carry):
        @pl.when(i >= 0)
        def _():
            attn_step(2 * i, (kb_b, qb_b, p_b, l_b), (p_a, l_a), (kb_a, qb_a))

        @pl.when(i < H // 2 - 1)
        def _():
            attn_step(2 * i + 1, (kb_a, qb_a, p_a, l_a), (p_b, l_b), (kb_b, qb_b))

        return carry

    with _scope('p2_loop'):
        lax.fori_loop(0, H // 2, attn_body, 0)

    l_last = jnp.sum(l_b[0:8, :] + l_b[8:16, :], axis=0, keepdims=True)
    lo = jnp.min(jnp.minimum(lmin_v[0:1, :], l_last))
    hi = jnp.max(jnp.maximum(lmax_v[0:1, :], l_last))
    safe = jnp.logical_and(lo >= L_MIN, hi <= L_MAX)

    @pl.when(jnp.logical_not(safe))
    def _():
        def exact(t, carry):
            h = t // NG
            cols = _rows(t % NG, TQ)
            q = _unpack(qt_v[h, 0:8, cols])
            s = jnp.dot(_unpack(k_v[h])[:, 0:DH], q, preferred_element_type=F32)
            p = jnp.exp2(s - jnp.max(s, axis=0, keepdims=True))
            p_b[:, cols] = _pack(p)
            l = jnp.sum(p.reshape(S // 8, 8, TQ), axis=0)
            l_b[0:8, cols] = l
            l_b[8:16, cols] = jnp.zeros((8, TQ), F32)
            o = jnp.dot(_unpack(vt_v[_rows(h, 8), :]), p.astype(BF16), preferred_element_type=F32)
            ot_v[_rows(h, DH), cols] = o * (1.0 / jnp.sum(l, axis=0, keepdims=True))
            return carry

        lax.fori_loop(0, H * NG, exact, 0)

    KA = D - 128
    zoff = pl.multiple_of(zero * 16, 16)

    def paced(r0):
        return pl.ds(zoff + r0, RC)

    NZ = FH // 128
    nch = T3 // RC
    md = {}

    def modrow(k):
        return jnp.concatenate([md[k * 4 + t] for t in range(4)], axis=1)

    def wo_rest(i):
        rows = pl.ds(i * T3, T3)
        ob = ot_v[pl.ds(KA, D - KA), rows].T.astype(BF16)
        return jnp.dot(ob, wo_v[pl.ds(KA, D - KA), :], preferred_element_type=F32)

    def front_chunk(i, yb, j):
        r0 = i * T3 + j * RC
        x1 = x1_v[paced(r0) if i > 0 else pl.ds(r0, RC), :] + modrow(0) * yb[j * RC:(j + 1) * RC]
        x1_v[pl.ds(r0, RC), :] = x1
        return (_ln(x1) * (1.0 + modrow(2)) + modrow(1)).astype(BF16)

    with _scope('p2_last'):
        wait(cp_mid)
        c = c_v[...].astype(F32)
        sc = jnp.broadcast_to(c * jax.nn.sigmoid(c), (16, D)).astype(BF16)
        bsp = bsp_v[0:S // 128, :].astype(F32)
        for i in range(S // 128):
            bcol_v[pl.ds(i * 128, 128), :] = jnp.broadcast_to(bsp[i:i + 1, :], (128, 128)).T
        last = pv_items(H - 1, p_b, l_b, track=False)
        ys = {}

        def mod_piece(t):
            mt = jnp.dot(sc, wmod_v[:, pl.ds(2 * D + t * 128, 128)], preferred_element_type=F32)
            md[t] = mt[0:1]
            if t >= 12:
                mod_v[0:8, pl.ds((t - 12) * 128, 128)] = mt[0:8]

        def wo_piece(i, kt):
            rows = pl.ds(i * 128, 128)
            oa = ot_v[pl.ds(kt * 128, 128), rows].T.astype(BF16)
            ya = jnp.dot(oa, wo_v[pl.ds(kt * 128, 128), :], preferred_element_type=F32)
            ys[i] = ya if kt == 0 else ya + ys[i]

        def x1_part(i):
            rows = pl.ds(i * 128, 128)
            x1_v[rows, :] = x_v[rows, :].astype(F32) + modrow(0) * ys.pop(i)

        for n, it in enumerate(last):
            it()
            if n % 4 == 0:
                mod_piece(n // 4)
            else:
                wo_piece(n // 4, n % 4 - 1)
            if n % 4 == 3 and n // 4 >= 3:
                for i in (range(4) if n // 4 == 3 else [n // 4]):
                    x1_part(i)
            if n == 47:
                yb = wo_rest(0)
                h2 = jnp.concatenate([front_chunk(0, yb, j) for j in range(nch)], axis=0)

    with _scope('p3'):
        for i in range(N3):
            rows = pl.ds(i * T3, T3)
            yb = wo_rest(i + 1) if i + 1 < N3 else None
            hparts = []
            for sl in range(2 * NZ):
                lhs = h2
                if sl == NZ + ZL:
                    tok = pltpu.bitcast(jnp.broadcast_to(jnp.max(rstd, axis=0, keepdims=True) * 0.0, (8, 128)), U32)
                    h32 = pltpu.bitcast(h2, U32)
                    lhs = _unpack(jnp.concatenate(
                        [jnp.concatenate([h32[0:8, 0:128] + tok, h32[0:8, 128:]], axis=1), h32[8:]], axis=0))
                zraw = jnp.dot(lhs, win_v[:, pl.ds(((sl + NZ) % (2 * NZ)) * 128, 128)], preferred_element_type=F32)
                zt = _gelu(zraw)
                if sl < NZ:
                    zr_v[rows, pl.ds(sl * 128, 128)] = zt
                    s1 = zt if sl == 0 else s1 + zt
                    s2 = zt * zt if sl == 0 else s2 + zt * zt
                    if sl == NZ - 1:
                        mean = jnp.sum(s1, axis=-1, keepdims=True) * (1.0 / FH)
                        var = jnp.sum(s2, axis=-1, keepdims=True) * (1.0 / FH) - mean * mean
                        rstd = lax.rsqrt(jnp.maximum(var, 0.0) + EPS)
                else:
                    z1_v[rows, pl.ds((sl - NZ) * 128, 128)] = zt
                    lo_s = NZ + ZL
                    if sl >= lo_s:
                        zr_v[pl.ds(S, 8), pl.ds(0, 128)] = zraw[0:8]
                        ns = 2 * NZ - lo_s
                        for j in range((sl - lo_s) * nch // ns, (sl - lo_s + 1) * nch // ns):
                            r0 = i * T3 + j * RC
                            g2 = zr_v[paced(r0), :]
                            z2_v[pl.ds(r0 // 2, RC // 2), :] = _pack(
                                (g2 - mean[j * RC:(j + 1) * RC]) * rstd[j * RC:(j + 1) * RC])
                if yb is not None and sl < FS:
                    x1_v[pl.ds(S, 8), pl.ds(0, 128)] = zraw[0:8]
                    for j in range(sl * nch // FS, (sl + 1) * nch // FS):
                        hparts.append(front_chunk(i + 1, yb, j))
            if yb is not None:
                h2 = jnp.concatenate(hparts, axis=0)

    NO = T4 // TO

    def out_copy(i):
        rows = _rows(i, TO)
        return pltpu.make_async_copy(x_v.at[rows, :], out_hbm.at[0, rows, :], sems.at[8])

    def out_body(i, carry):
        rows = _rows(i, T4)
        g = jnp.dot(wsp_v[rows, :], _unpack(z2_v[...]), preferred_element_type=F32)
        bc = bcol_v[rows, :]
        g = g + jnp.concatenate([bc] * (FH // 128), axis=1)
        u = (z1_v[rows, :] * g).astype(BF16)
        for t in range(NO):
            hrows = _rows(NO * i + t, TO)
            y2 = jnp.dot(u[t * TO:(t + 1) * TO], wout_v[...], preferred_element_type=F32)
            x_v[hrows, :] = (x1_v[hrows, :] + mod_v[0:1, :] * y2).astype(BF16)
            out_copy(NO * i + t).start()
        return carry

    with _scope('p4'):
        wait(cp_end)
        lax.fori_loop(0, N4, out_body, 0)
        for i in range(NO * N4):
            out_copy(i).wait()


@jax.jit
def pallas_adaLN_cond__softmax_full_mha__mixer_gmlp__prompt_kernel(
    A_x: jax.Array,
    A_wqkv: jax.Array,
    A_wo: jax.Array,
    B_x: jax.Array,
    B_w_in: jax.Array,
    B_w_sp: jax.Array,
    B_b_sp: jax.Array,
    B_w_out: jax.Array,
    c: jax.Array,
    w_mod: jax.Array,
):
    del B_x
    any_spec = pl.BlockSpec(memory_space=pl.ANY)
    scratch = [
        pltpu.VMEM((S, D), BF16),
        pltpu.VMEM((D, 3 * D), BF16),
        pltpu.VMEM((D, D), BF16),
        pltpu.VMEM((D, F), BF16),
        pltpu.VMEM((S, S), BF16),
        pltpu.VMEM((FH, D), BF16),
        pltpu.VMEM((D, 6 * D), BF16),
        pltpu.VMEM((32, D), F32),
        pltpu.VMEM((D, D), U32),
        pltpu.VMEM((S // 2, D), U32),
        pltpu.VMEM((S // 2, D), U32),
        pltpu.VMEM((H, S // 2, 128), U32),
        pltpu.VMEM((H, DH, S), U32),
        pltpu.VMEM((D // 2, S), U32),
        pltpu.VMEM((D, S), F32),
        pltpu.VMEM((S // 2, S), U32),
        pltpu.VMEM((S // 2, S), U32),
        pltpu.VMEM((16, S), F32),
        pltpu.VMEM((16, S), F32),
        pltpu.VMEM((8, S), F32),
        pltpu.VMEM((8, S), F32),
        pltpu.VMEM((NB * 128, D), F32),
        pltpu.VMEM((H + 2, QT_ROWS, 128), F32),
        pltpu.VMEM((DH, NB * 128, 128), F32),
        pltpu.VMEM((DH, NB * 128, 128), F32),
        pltpu.VMEM((QB_ROWS, TQ), F32),
        pltpu.VMEM((QB_ROWS, TQ), F32),
        pltpu.VMEM((S + 32, D), F32),
        pltpu.VMEM((S, FH), F32),
        pltpu.VMEM((S + 128, FH), F32),
        pltpu.VMEM((S // 2, FH), U32),
        pltpu.VMEM((S, 128), F32),
        pltpu.VMEM((248, 128), BF16),
        pltpu.VMEM((1, D), BF16),
        pltpu.SemaphoreType.DMA((11,)),
    ]
    return pl.pallas_call(
        _kernel,
        out_shape=jax.ShapeDtypeStruct((1, S, D), BF16),
        in_specs=[any_spec] * 9,
        out_specs=any_spec,
        scratch_shapes=scratch,
        compiler_params=pltpu.CompilerParams(vmem_limit_bytes=124 * 1024 * 1024),
        name="fused_block",
    )(A_x, A_wqkv, A_wo, B_w_in, B_w_sp, B_b_sp.reshape(S // 128, 128), B_w_out, c, w_mod)
```
